```python
import jax
import jax.numpy as jnp

def _softmax(x, axis=-1):
    return jax.nn.softmax(x, axis=axis)

def _gelu(x):
    return jax.nn.gelu(x, approximate=True)

def _silu(x):
    return jax.nn.silu(x)

def _sigmoid(x):
    return jax.nn.sigmoid(x)

def _layernorm(x, axis=-1, eps=1e-05):
    m = jnp.mean(x, axis=axis, keepdims=True)
    v = jnp.var(x, axis=axis, keepdims=True)
    return (x - m) / jnp.sqrt(v + eps)

def _scatter_add(tgt, idx, src, axis=0):
    return tgt.at[idx].add(src)

def _segment_sum(src, seg, n):
    return jax.ops.segment_sum(src, seg, n)

class _Rng:

    def __init__(self, key):
        self._k = key

    def _next(self):
        self._k, sub = jax.random.split(self._k)
        return sub

    def normal(self, shape):
        return jax.random.normal(self._next(), shape, dtype=jnp.bfloat16)

    def randint(self, lo, hi, shape):
        return jax.random.randint(self._next(), shape, lo, hi, dtype=jnp.int32)

    def uniform(self, shape, lo=0.0, hi=1.0):
        return jax.random.uniform(self._next(), shape, jnp.bfloat16, lo, hi)

    def permutation(self, n):
        return jax.random.permutation(self._next(), n)
kernel_name = 'interleave_layers__memory_aug_recurrent_mem_tr__spectral_gfnet__prompt'

def setup_inputs():
    _rng = _Rng(jax.random.key(int.from_bytes(__import__("os").urandom(4), "little")))
    _w = lambda a: (lambda t: t.astype(jnp.bfloat16) if jnp.issubdtype(t.dtype, jnp.floating) else t)(jnp.asarray(a))

    def _A_setup():
        B, S, Dm = (1, 2048, 640)
        H, Dh = (32, 128)
        M, seg = (8, 32)
        seg = min(seg, S)
        S = S // seg * seg
        return {'x': _w((lambda *s: _rng.normal(s) * 0.05)(B, S, Dm)), 'mem0': _w((lambda *s: _rng.normal(s) * 0.05)(B, M, Dm)), 'Wq': _w((lambda *s: _rng.normal(s) * 0.05)(Dm, H, Dh) * Dm ** (-0.5)), 'Wk': _w((lambda *s: _rng.normal(s) * 0.05)(Dm, H, Dh) * Dm ** (-0.5)), 'Wv': _w((lambda *s: _rng.normal(s) * 0.05)(Dm, H, Dh) * Dm ** (-0.5)), 'Wo': _w((lambda *s: _rng.normal(s) * 0.05)(H, Dh, Dm) * (H * Dh) ** (-0.5)), 'seg_len': seg}
    _A_in = _A_setup()

    def _B_setup():
        B, S, D = (1, 2048, 640)
        Df = D // 2 + 1
        return {'x': _w((lambda *s: _rng.normal(s) * 0.05)(B, S, D)), 'w_r': _w((lambda *s: _rng.normal(s) * 0.05)(S, Df) * 0.02), 'w_i': _w((lambda *s: _rng.normal(s) * 0.05)(S, Df) * 0.02)}
    _B_in = _B_setup()
    return {'A_x': _A_in['x'], 'A_mem0': _A_in['mem0'], 'A_Wq': _A_in['Wq'], 'A_Wk': _A_in['Wk'], 'A_Wv': _A_in['Wv'], 'A_Wo': _A_in['Wo'], 'A_seg_len': _A_in['seg_len'], 'B_x': _B_in['x'], 'B_w_r': _B_in['w_r'], 'B_w_i': _B_in['w_i']}

def reference(A_x, A_mem0, A_Wq, A_Wk, A_Wv, A_Wo, A_seg_len, B_x, B_w_r, B_w_i):

    def _A_ref(x, mem0, Wq, Wk, Wv, Wo, seg_len):
        B, S, Dm = x.shape
        H, Dh = (Wq.shape[1], Wq.shape[2])
        M = mem0.shape[1]
        scale = Dh ** (-0.5)
        n_seg = S // seg_len
        L = M + seg_len
        idx = jnp.arange(L)
        mask = (idx[:, None] < M) | (idx[:, None] >= idx[None, :])
        mem = mem0
        outs = []
        for s in range(n_seg):
            xs = x[:, s * seg_len:(s + 1) * seg_len, :].copy()
            h = jnp.concatenate([mem, xs], axis=1)
            q = jnp.einsum('btd,dhe->bhte', h, Wq)
            k = jnp.einsum('btd,dhe->bhte', h, Wk)
            v = jnp.einsum('btd,dhe->bhte', h, Wv)
            scores = jnp.einsum('bhqe,bhke->bhqk', q, k) * scale
            scores = jnp.where(mask[None, None], scores, -1000000000.0)
            p = _softmax(scores, axis=-1)
            o = jnp.einsum('bhqk,bhke->bhqe', p, v)
            o = jnp.einsum('bhte,hed->btd', o, Wo)
            mem = o[:, :M, :].copy()
            outs.append(o[:, M:, :])
        return jnp.concatenate(outs, axis=1)

    def _B_ref(x, w_r, w_i):
        B, S, D = x.shape
        X = (lambda x, axes=(-2, -1): jnp.fft.rfft2(x.astype(jnp.float32), axes=axes))(x, axes=(-2, -1))
        W = w_r + 1j * w_i
        X = X * W
        y = (lambda x, s, axes=(-2, -1): jnp.fft.irfft2(x, s=s, axes=axes).astype(jnp.bfloat16))(X, (S, D), axes=(-2, -1))
        return y
    x = A_x
    x = x + _A_ref(_layernorm(x, axis=-1), A_mem0, A_Wq, A_Wk, A_Wv, A_Wo, A_seg_len)
    x = x + _B_ref(_layernorm(x, axis=-1), B_w_r, B_w_i)
    x = x + _A_ref(_layernorm(x, axis=-1), A_mem0, A_Wq, A_Wk, A_Wv, A_Wo, A_seg_len)
    x = x + _B_ref(_layernorm(x, axis=-1), B_w_r, B_w_i)
    return x
```

```python
import functools

import numpy as np
import jax
import jax.numpy as jnp
import jax.experimental.pallas as pl
import jax.experimental.pallas.tpu as pltpu

F32 = jnp.float32
BF16 = jnp.bfloat16
U32 = jnp.uint32

S, D, DF = 2048, 640, 321
H, DH = 32, 128
M, SEG = 8, 32
L = M + SEG
NSEG = S // SEG
G = 4
NG = H // G
R = 16
EPS = 1e-5

_NN = (((1,), (0,)), ((), ()))
_NT = (((1,), (1,)), ((), ()))


def _freq_classes():
    k0 = np.arange(0, DF, 5)
    k14 = np.concatenate([np.arange(1, DF, 5), np.arange(4, DF, 5)])
    k23 = np.concatenate([np.arange(2, DF, 5), np.arange(3, DF, 5)])
    return k0, k14, k23


def _tables():
    k0, k14, k23 = _freq_classes()
    b = np.arange(128)

    def ang(k):
        return 2.0 * np.pi * ((b[:, None] * k[None, :]) % D) / D

    f0 = np.zeros((128, 256))
    f0[:, :65] = np.cos(ang(k0))
    f0[:, 128:128 + 65] = -np.sin(ang(k0))
    g0 = np.zeros((256, 128))
    c0 = np.where((k0 == 0) | (k0 == D // 2), 1.0, 2.0)
    g0[:65] = (np.cos(ang(k0)) * c0).T
    g0[128:128 + 65] = (-np.sin(ang(k0)) * c0).T
    sgn = np.concatenate([np.ones(64), -np.ones(64)])[None, :]
    fs, gs = [], []
    for k in (k14, k23):
        c, s = np.cos(ang(k)), np.sin(ang(k))
        f = np.block([[c, -s], [s * sgn, c * sgn]])
        fs.append(f)
        gs.append(2.0 * f.T)
    rowf = np.concatenate([f0, fs[0], fs[1]], axis=0)
    rowg = np.concatenate([np.concatenate([g0, np.zeros((256, 128))], 1),
                           gs[0], gs[1]], axis=0)

    colf = np.zeros((R, 256, 256))
    colg = np.zeros((R, 256, 256))
    for k1 in range(R):
        a = 2.0 * np.pi * (((k1 + R * b)[:, None] * b[None, :]) % S) / S
        c, s = np.cos(a), np.sin(a)
        colf[k1, :128, 0::2], colf[k1, :128, 1::2] = c, s
        colf[k1, 128:, 0::2], colf[k1, 128:, 1::2] = -s, c
        colg[k1, :128, 0::2], colg[k1, :128, 1::2] = c.T, -s.T
        colg[k1, 128:, 0::2], colg[k1, 128:, 1::2] = s.T, c.T

    pcol = np.zeros((DF, 384))
    for t, k in enumerate((k0, k14, k23)):
        pcol[k, 128 * t + np.arange(len(k))] = 1.0
    prow = np.zeros((128, 128))
    prow[(b % R) * 8 + b // R, b] = 1.0
    bf = lambda t: np.asarray(t, np.float32).astype(BF16)
    return bf(rowf), bf(rowg), bf(colf), bf(colg), bf(pcol.T), bf(prow)


_C1, _C2 = float(np.cos(2 * np.pi / 5)), float(np.cos(4 * np.pi / 5))
_S1, _S2 = float(np.sin(2 * np.pi / 5)), float(np.sin(4 * np.pi / 5))
_C8 = float(np.sqrt(0.5))
_C16, _S16 = float(np.cos(np.pi / 8)), float(np.sin(np.pi / 8))


def _dot(a, b, dn=_NN):
    return jax.lax.dot_general(a, b, dn, preferred_element_type=F32)


def _bf(u):
    return pltpu.bitcast(u, BF16)


def _pack(re, im):
    return pltpu.bitcast(pltpu.pack_elementwise([re, im], packed_dtype=BF16), U32)


def _layernorm(x):
    m = jnp.mean(x, axis=-1, keepdims=True)
    xc = x - m
    v = jnp.mean(xc * xc, axis=-1, keepdims=True)
    return xc * jax.lax.rsqrt(v + EPS)


def _dft4(x0, x1, x2, x3):
    ar, ai = x0[0] + x2[0], x0[1] + x2[1]
    br, bi = x0[0] - x2[0], x0[1] - x2[1]
    cr, ci = x1[0] + x3[0], x1[1] + x3[1]
    dr, di = x1[0] - x3[0], x1[1] - x3[1]
    return ((ar + cr, ai + ci), (br + di, bi - dr), (ar - cr, ai - ci), (br - di, bi + dr))


def _tw16(x, p):
    r, i = x
    if p == 0:
        return x
    if p == 4:
        return (i, -r)
    if p == 2:
        return ((r + i) * _C8, (i - r) * _C8)
    if p == 6:
        return ((i - r) * _C8, (r + i) * (-_C8))
    c, s = {1: (_C16, _S16), 3: (_S16, _C16), 9: (-_C16, -_S16)}[p]
    return (r * c + i * s, i * c - r * s)


def _dft16(x):
    t = [_dft4(x[j], x[j + 4], x[j + 8], x[j + 12]) for j in range(4)]
    out = [None] * 16
    for k in range(4):
        y = _dft4(*[_tw16(t[j][k], j * k) for j in range(4)])
        for q in range(4):
            out[k + 4 * q] = y[q]
    return out


def _row_fwd(x, rowf):
    h = _layernorm(x)
    a = [h[:, 128 * i:128 * (i + 1)] for i in range(5)]
    p1, m1, p2, m2 = a[1] + a[4], a[4] - a[1], a[2] + a[3], a[3] - a[2]
    u0 = a[0] + p1 + p2
    u1 = jnp.concatenate([a[0] + _C1 * p1 + _C2 * p2, _S1 * m1 + _S2 * m2], axis=1)
    u2 = jnp.concatenate([a[0] + _C2 * p1 + _C1 * p2, _S2 * m1 - _S1 * m2], axis=1)
    return jnp.concatenate([_dot(u0, _bf(rowf[0:64])),
                            _dot(u1, _bf(rowf[64:192])),
                            _dot(u2, _bf(rowf[192:320]))], axis=1)


def _row_inv(z, rowg):
    t0 = _dot(z[:, 0:256], _bf(rowg[0:128, 0:128]))
    t1 = _dot(z[:, 256:512], _bf(rowg[128:256]))
    t2 = _dot(z[:, 512:768], _bf(rowg[256:384]))
    t1r, t1i, t2r, t2i = t1[:, :128], t1[:, 128:], t2[:, :128], t2[:, 128:]
    a1, b1 = t0 + _C1 * t1r + _C2 * t2r, _S1 * t1i + _S2 * t2i
    a2, b2 = t0 + _C2 * t1r + _C1 * t2r, _S2 * t1i - _S1 * t2i
    return jnp.concatenate([t0 + t1r + t2r, a1 - b1, a2 - b2, a2 + b2, a1 + b1], axis=1)


def _attention_step(h, wqkv, wo):
    row = jax.lax.broadcasted_iota(jnp.int32, (L, L), 0)
    col = jax.lax.broadcasted_iota(jnp.int32, (L, L), 1)
    mask = (row < M) | (row >= col)

    def scores(t):
        res = []
        for i in range(G):
            q = t[:, 384 * i:384 * i + 128]
            k = t[:, 384 * i + 128:384 * i + 256].astype(BF16)
            v = t[:, 384 * i + 256:384 * i + 384].astype(BF16)
            sc = jnp.where(mask, _dot(q, k, _NT) * (DH ** -0.5), -1e9)
            p = jnp.exp(sc - jnp.max(sc, axis=-1, keepdims=True))
            res.append((p, 1.0 / jnp.sum(p, axis=-1, keepdims=True), v))
        return res

    qkv, prob, out, acc = {}, {}, {}, None
    for g in range(NG + 3):
        if g < NG:
            qkv[g] = _dot(h, _bf(wqkv[g]))
        if 0 <= g - 1 < NG:
            prob[g - 1] = scores(qkv.pop(g - 1))
        if 0 <= g - 2 < NG:
            out[g - 2] = jnp.concatenate([_dot(p, v) * r for p, r, v in prob.pop(g - 2)], axis=1)
        if 0 <= g - 3 < NG:
            d = _dot(out.pop(g - 3), _bf(wo[g - 3]))
            acc = d if acc is None else acc + d
    return acc


def _kernel(x_hbm, mem0_hbm, rowf_hbm, rowg_hbm, pcol_hbm, prow_hbm,
            wq_hbm, wk_hbm, wv_hbm, wo_hbm, wr_hbm, wi_hbm, colf_hbm, colg_hbm,
            out_ref,
            x_ref, mem0_ref, rowf_in, rowg_in, pcol_ref, prow_ref,
            wqkv, wo, stage, wo_st, wr_st, wi_st, colf, colg, rowf, rowg,
            xa, xf, yp, wp, sem_w, sem_o, sem_c):
    small = [pltpu.make_async_copy(a, b, sem_c.at[i]) for i, (a, b) in enumerate((
        (pcol_hbm, pcol_ref), (prow_hbm, prow_ref), (wr_hbm, wr_st), (wi_hbm, wi_st),
        (rowf_hbm, rowf_in), (mem0_hbm, mem0_ref), (x_hbm, x_ref),
        (rowg_hbm, rowg_in), (colf_hbm, colf), (colg_hbm, colg)))]
    fil, inp, tab = small[:4], small[4:7], small[7:]
    pairs = [[pltpu.make_async_copy(w.bitcast(U32).at[:, p, :], stage.at[j, p], sem_w.at[j, p])
              for j, w in enumerate((wq_hbm, wk_hbm, wv_hbm))] for p in range(H // 2)]
    wos = [pltpu.make_async_copy(wo_hbm.at[g], wo_st.at[g], sem_o.at[g]) for g in range(NG)]
    for c in fil + [c for cs in pairs for c in cs] + wos + inp + tab:
        c.start()

    for c in fil:
        c.wait()

    def filter_block(j, _):
        cols = pl.ds(pl.multiple_of(j * 128, 128), 128)
        dst = pl.ds(pl.multiple_of(j * 8, 8), 8)
        for part, st in enumerate((wr_st, wi_st)):
            t = _dot(pcol_ref[...], st[:, cols]).astype(BF16)
            t = _dot(prow_ref[...], t, _NT) * (1.0 / (S * D))
            for c in range(3):
                lo = 256 * c + 128 * part
                wp[:, dst, lo:lo + 128] = t[:, 128 * c:128 * (c + 1)].reshape(R, 8, 128)
    jax.lax.fori_loop(0, S // 128, filter_block, None)

    for p in range(H // 2):
        for j in range(3):
            pairs[p][j].wait()
            a = stage[j, p, pl.ds(0, D // 2, stride=2), :]
            b = stage[j, p, pl.ds(1, D // 2, stride=2), :]
            for e, w in enumerate(((a & 0xFFFF) | (b << 16),
                                   (a >> 16) | (b & np.uint32(0xFFFF0000)))):
                g, i = divmod(2 * p + e, G)
                lo = 384 * i + 128 * j
                wqkv[g, :, lo:lo + 128] = w
    for g in range(NG):
        wos[g].wait()
        wo[g] = pltpu.bitcast(wo_st[g], U32)
    for c in inp:
        c.wait()
    rowf[...] = pltpu.bitcast(rowf_in[...], U32)

    def seg_rows(s):
        return pl.ds(pl.multiple_of(s * SEG, SEG), SEG)

    def a_block(load):
        x0 = load(0)

        def step(s, carry):
            mem, xs, hs, xprev = carry
            xf[seg_rows(jnp.maximum(s - 1, 0)), :] = _row_fwd(xprev, rowf)
            xn = load(jnp.minimum(s + 1, NSEG - 1))
            o = _attention_step(jnp.concatenate([mem, hs], axis=0), wqkv, wo)
            xo = xs + o[M:]
            xa[seg_rows(s), :] = xo
            return o[:M], xn, _layernorm(xn), xo

        init = (mem0_ref[...].astype(F32), x0, _layernorm(x0), x0)
        last = jax.lax.fori_loop(0, NSEG, step, init)[3]
        xf[S - SEG:, :] = _row_fwd(last, rowf)

    def b_block():
        def radix_fwd(i, _):
            for c in range(3):
                x = [(xf[pl.ds(pl.multiple_of(128 * n + 8 * i, 8), 8), 256 * c:256 * c + 128],
                      xf[pl.ds(pl.multiple_of(128 * n + 8 * i, 8), 8), 256 * c + 128:256 * c + 256])
                     for n in range(R)]
                for k, (re, im) in enumerate(_dft16(x)):
                    yp[k, pl.ds(pl.multiple_of(8 * i, 8), 8), 128 * c:128 * (c + 1)] = _pack(re, im)
        jax.lax.fori_loop(0, 16, radix_fwd, None)

        def spectral(k, _):
            x = _dot(colf[k], _bf(yp[k]))
            z = []
            for c in range(3):
                xr, xi = x[:128, 128 * c:128 * (c + 1)], x[128:, 128 * c:128 * (c + 1)]
                wr, wi = wp[k, :, 256 * c:256 * c + 128], wp[k, :, 256 * c + 128:256 * c + 256]
                z.append(_pack(xr * wr - xi * wi, xr * wi + xi * wr))
            v = _dot(colg[k], _bf(jnp.concatenate(z, axis=1)))
            rows = pl.ds(pl.multiple_of(128 * k, 128), 128)
            for c in range(3):
                xf[rows, 256 * c:256 * c + 128] = v[:128, 128 * c:128 * (c + 1)]
                xf[rows, 256 * c + 128:256 * c + 256] = v[128:, 128 * c:128 * (c + 1)]
        jax.lax.fori_loop(0, R, spectral, None)

        def radix_inv(i, _):
            for c in range(3):
                idx = [pl.ds(pl.multiple_of(128 * n + 8 * i, 8), 8) for n in range(R)]
                re, im = slice(256 * c, 256 * c + 128), slice(256 * c + 128, 256 * c + 256)
                y = _dft16([(xf[r, im], xf[r, re]) for r in idx])
                for r, (yi, yr) in zip(idx, y):
                    xf[r, re] = yr
                    xf[r, im] = yi
        jax.lax.fori_loop(0, 16, radix_inv, None)

    def after_b(rows):
        return xa[rows, :] + _row_inv(xf[rows, :], rowg)

    a_block(lambda s: x_ref[seg_rows(s), :].astype(F32))
    for c in tab:
        c.wait()
    rowg[...] = pltpu.bitcast(rowg_in[...], U32)
    b_block()
    a_block(lambda s: after_b(seg_rows(s)))
    b_block()

    def finish(j, _):
        rows = pl.ds(pl.multiple_of(j * 128, 128), 128)
        out_ref[rows, :] = after_b(rows).astype(out_ref.dtype)
    jax.lax.fori_loop(0, S // 128, finish, None)


@functools.partial(jax.jit, static_argnames=("A_seg_len",))
def pallas_interleave_layers__memory_aug_recurrent_mem_tr__spectral_gfnet__prompt_kernel(
    A_x: jax.Array,
    A_mem0: jax.Array,
    A_Wq: jax.Array,
    A_Wk: jax.Array,
    A_Wv: jax.Array,
    A_Wo: jax.Array,
    A_seg_len: int,
    B_x: jax.Array,
    B_w_r: jax.Array,
    B_w_i: jax.Array,
):
    assert A_seg_len == SEG and A_x.shape == (1, S, D) and A_mem0.shape == (1, M, D)
    assert A_Wq.shape == (D, H, DH) and B_w_r.shape == (S, DF)
    rowf, rowg, colf, colg, pcol, prow = _tables()
    vmem = pl.BlockSpec(memory_space=pltpu.VMEM)
    hbm = pl.BlockSpec(memory_space=pltpu.HBM)
    out = pl.pallas_call(
        _kernel,
        out_shape=jax.ShapeDtypeStruct((S, D), A_x.dtype),
        in_specs=[hbm] * 14,
        out_specs=vmem,
        scratch_shapes=[
            pltpu.VMEM((S, D), BF16),
            pltpu.VMEM((M, D), BF16),
            pltpu.VMEM((640, 256), BF16),
            pltpu.VMEM((768, 256), BF16),
            pltpu.VMEM((384, DF), BF16),
            pltpu.VMEM((128, 128), BF16),
            pltpu.VMEM((NG, D // 2, 3 * G * DH), U32),
            pltpu.VMEM((NG, G * DH // 2, D), U32),
            pltpu.VMEM((3, H // 2, D, DH), U32),
            pltpu.VMEM((NG, G * DH, D), BF16),
            pltpu.VMEM((DF, S), BF16),
            pltpu.VMEM((DF, S), BF16),
            pltpu.VMEM((R, 256, 256), BF16),
            pltpu.VMEM((R, 256, 256), BF16),
            pltpu.VMEM((320, 256), U32),
            pltpu.VMEM((384, 256), U32),
            pltpu.VMEM((S, D), F32),
            pltpu.VMEM((S, 768), F32),
            pltpu.VMEM((R, 128, 384), U32),
            pltpu.VMEM((R, 128, 768), F32),
            pltpu.SemaphoreType.DMA((3, H // 2)),
            pltpu.SemaphoreType.DMA((NG,)),
            pltpu.SemaphoreType.DMA((10,)),
        ],
        compiler_params=pltpu.CompilerParams(vmem_limit_bytes=110 * 2 ** 20),
    )(A_x.reshape(S, D), A_mem0.reshape(M, D), rowf, rowg, pcol, prow,
      A_Wq, A_Wk, A_Wv, A_Wo.reshape(NG, G * DH, D), B_w_r.T, B_w_i.T, colf, colg)
    return out.reshape(A_x.shape)
```

```python
import functools

import numpy as np
import jax
import jax.numpy as jnp
import jax.experimental.pallas as pl
import jax.experimental.pallas.tpu as pltpu

F32 = jnp.float32
BF16 = jnp.bfloat16
U32 = jnp.uint32

S, D, DF = 2048, 640, 321
H, DH = 32, 128
M, SEG = 8, 32
L = M + SEG
NSEG = S // SEG
import os
LB, LC, N1, N2, *SIDE = map(int, os.environ.get('KP', '1,2,4,6,99,4').split(','))
UN = int(os.environ.get('UN', '2'))
BLAG = int(os.environ.get('BLAG', '2'))
NP = H // 2
PRE = 8
R = 32
EPS = 1e-5

_NN = (((1,), (0,)), ((), ()))
_NT = (((1,), (1,)), ((), ()))


def _freq_classes():
    k0 = np.arange(0, DF, 5)
    k14 = np.concatenate([np.arange(1, DF, 5), np.arange(4, DF, 5)])
    k23 = np.concatenate([np.arange(2, DF, 5), np.arange(3, DF, 5)])
    return k0, k14, k23


def _tables():
    k0, k14, k23 = _freq_classes()
    b = np.arange(128)

    def ang(k):
        return 2.0 * np.pi * ((b[:, None] * k[None, :]) % D) / D

    f0 = np.zeros((128, 256))
    f0[:, :65] = np.cos(ang(k0))
    f0[:, 128:128 + 65] = -np.sin(ang(k0))
    g0 = np.zeros((256, 128))
    c0 = np.where((k0 == 0) | (k0 == D // 2), 1.0, 2.0)
    g0[:65] = (np.cos(ang(k0)) * c0).T
    g0[128:128 + 65] = (-np.sin(ang(k0)) * c0).T
    sgn = np.concatenate([np.ones(64), -np.ones(64)])[None, :]
    fs, gs = [], []
    for k in (k14, k23):
        c, s = np.cos(ang(k)), np.sin(ang(k))
        f = np.block([[c, -s], [s * sgn, c * sgn]])
        fs.append(f)
        gs.append(2.0 * f.T)
    rowf = np.concatenate([f0, fs[0], fs[1]], axis=0)
    rowg = np.concatenate([np.concatenate([g0, np.zeros((256, 128))], 1),
                           gs[0], gs[1]], axis=0)

    n2 = np.arange(64)
    colf = np.zeros((R, 128, 128))
    colg = np.zeros((R, 128, 128))
    for k1 in range(R):
        k2 = n2 ^ (4 * (k1 % 2))
        a = 2.0 * np.pi * (((k1 + R * k2)[:, None] * n2[None, :]) % S) / S
        c, s = np.cos(a), np.sin(a)
        colf[k1, :64, 0::2], colf[k1, :64, 1::2] = c, s
        colf[k1, 64:, 0::2], colf[k1, 64:, 1::2] = -s, c
        colg[k1, :64, 0::2], colg[k1, :64, 1::2] = c.T, -s.T
        colg[k1, 64:, 0::2], colg[k1, 64:, 1::2] = s.T, c.T

    prow = np.zeros((2, 128, 128))
    k1, i = b % R, b // R
    for e in range(2):
        prow[e, 8 * (k1 // 2) + 4 * ((k1 + e) % 2) + i, b] = 1.0
    tw = np.concatenate([np.cos(2 * np.pi * np.arange(R) / R), np.sin(2 * np.pi * np.arange(R) / R)])

    def words(t):
        u = np.asarray(t, np.float32).astype(BF16).view(np.uint16).astype(np.uint32)
        return u[..., 0::2, :] | (u[..., 1::2, :] << np.uint32(16))

    return words(rowf), words(rowg), words(colf), words(colg), words(prow), tw.astype(np.float32)


_C1, _C2 = float(np.cos(2 * np.pi / 5)), float(np.cos(4 * np.pi / 5))
_S1, _S2 = float(np.sin(2 * np.pi / 5)), float(np.sin(4 * np.pi / 5))
_C8 = float(np.sqrt(0.5))


def _dot(a, b, dn=_NN):
    return jax.lax.dot_general(a, b, dn, preferred_element_type=F32)


def _bf(u):
    return pltpu.bitcast(u, BF16)


def _pack(re, im):
    return pltpu.bitcast(pltpu.pack_elementwise([re, im], packed_dtype=BF16), U32)


def _layernorm(x):
    m = jnp.mean(x, axis=-1, keepdims=True)
    xc = x - m
    v = jnp.mean(xc * xc, axis=-1, keepdims=True)
    return xc * jax.lax.rsqrt(v + EPS)


def _dft4(x0, x1, x2, x3):
    ar, ai = x0[0] + x2[0], x0[1] + x2[1]
    br, bi = x0[0] - x2[0], x0[1] - x2[1]
    cr, ci = x1[0] + x3[0], x1[1] + x3[1]
    dr, di = x1[0] - x3[0], x1[1] - x3[1]
    return ((ar + cr, ai + ci), (br + di, bi - dr), (ar - cr, ai - ci), (br - di, bi + dr))


def _dft8(x):
    e = _dft4(*x[0::2])
    o = _dft4(*x[1::2])
    o1 = ((o[1][0] + o[1][1]) * _C8, (o[1][1] - o[1][0]) * _C8)
    o3 = ((o[3][1] - o[3][0]) * _C8, (o[3][0] + o[3][1]) * _C8)
    return [(e[0][0] + o[0][0], e[0][1] + o[0][1]), (e[1][0] + o1[0], e[1][1] + o1[1]),
            (e[2][0] + o[2][1], e[2][1] - o[2][0]), (e[3][0] + o3[0], e[3][1] - o3[1]),
            (e[0][0] - o[0][0], e[0][1] - o[0][1]), (e[1][0] - o1[0], e[1][1] - o1[1]),
            (e[2][0] - o[2][1], e[2][1] + o[2][0]), (e[3][0] - o3[0], e[3][1] + o3[1])]


def _rotate(z, c, s):
    res = []
    for t in range(3):
        re, im = z[:, 256 * t:256 * t + 128], z[:, 256 * t + 128:256 * t + 256]
        res += [re * c - im * s, im * c + re * s]
    return jnp.concatenate(res, axis=1)


def _row_fwd(x, rowf):
    h = _layernorm(x)
    a = [h[:, 128 * i:128 * (i + 1)] for i in range(5)]
    p1, m1, p2, m2 = a[1] + a[4], a[4] - a[1], a[2] + a[3], a[3] - a[2]
    u0 = a[0] + p1 + p2
    u1 = jnp.concatenate([a[0] + _C1 * p1 + _C2 * p2, _S1 * m1 + _S2 * m2], axis=1)
    u2 = jnp.concatenate([a[0] + _C2 * p1 + _C1 * p2, _S2 * m1 - _S1 * m2], axis=1)
    return jnp.concatenate([_dot(u0, _bf(rowf[0:64])),
                            _dot(u1, _bf(rowf[64:192])),
                            _dot(u2, _bf(rowf[192:320]))], axis=1)


def _row_inv(z, rowg):
    t0 = _dot(z[:, 0:256], _bf(rowg[0:128, 0:128]))
    t1 = _dot(z[:, 256:512], _bf(rowg[128:256]))
    t2 = _dot(z[:, 512:768], _bf(rowg[256:384]))
    t1r, t1i, t2r, t2i = t1[:, :128], t1[:, 128:], t2[:, :128], t2[:, 128:]
    a1, b1 = t0 + _C1 * t1r + _C2 * t2r, _S1 * t1i + _S2 * t2i
    a2, b2 = t0 + _C2 * t1r + _C1 * t2r, _S2 * t1i - _S1 * t2i
    return jnp.concatenate([t0 + t1r + t2r, a1 - b1, a2 - b2, a2 + b2, a1 + b1], axis=1)


def _schedule():
    order, d = [], 0
    for g in range(NP + LC):
        if g < NP:
            order.append(("qkv", g))
        else:
            for _ in range(N1 if g == NP else N2):
                order.append(("wo", d))
                d += 1
        if 0 <= g - LB < NP:
            order.append(("qk", g - LB))
        if 0 <= g - LC < NP:
            order.append(("pv", g - LC))
        order += [("side", i) for i, pos in enumerate(SIDE) if pos == g]
    order += [("wo", g) for g in range(d, NP)]
    return order + [("side", i) for i, pos in enumerate(SIDE) if pos == 99]


def _attention_step(h, wqkv, wo, pre, side):
    row = jax.lax.broadcasted_iota(jnp.int32, (L, L), 0)
    col = jax.lax.broadcasted_iota(jnp.int32, (L, L), 1)
    mask = (row < M) | (row >= col)

    def project(g):
        if pre is None:
            return _dot(h, _bf(wqkv[g]))
        qk = jnp.concatenate([_dot(h[:L - PRE], _bf(wqkv[g, :, :512])), pre(g)], axis=0)
        return jnp.concatenate([qk, _dot(h, _bf(wqkv[g, :, 512:]))], axis=1)

    def scores(t):
        res = []
        for i in range(2):
            q = t[:, 128 * i:128 * i + 128]
            k = t[:, 128 * i + 256:128 * i + 384].astype(BF16)
            v = t[:, 128 * i + 512:128 * i + 640].astype(BF16)
            sc = jnp.where(mask, _dot(q, k, _NT) * (DH ** -0.5), -1e9)
            p = jnp.exp(sc - jnp.max(sc, axis=-1, keepdims=True))
            res.append((p, 1.0 / jnp.sum(p, axis=-1, keepdims=True), v))
        return res

    qkv, prob, out, acc = {}, {}, {}, None
    for op, g in _schedule():
        if op == "qkv":
            qkv[g] = project(g)
        elif op == "qk":
            prob[g] = scores(qkv.pop(g))
        elif op == "pv":
            out[g] = jnp.concatenate([_dot(p, v) * r for p, r, v in prob.pop(g)], axis=1)
        elif op == "side":
            side[g]()
        else:
            d = _dot(out.pop(g), _bf(wo[g]))
            acc = d if acc is None else acc + d
    return acc


def _kernel(tw, x_hbm, mem0_hbm, rowf_hbm, rowg_hbm, prow_hbm, colf_hbm, colg_hbm,
            wq_hbm, wk_hbm, wv_hbm, wo_hbm, wr_hbm, wi_hbm,
            out_hbm,
            x_ref, xq_ref, mem0_ref, rowf, rowg, prow, colf, colg,
            wqkv, wo, stage, wo_st, wr_st, wi_st, wf, hq, qk_pre,
            xa, cf, ef, yp, wp, obuf, sem_w, sem_c, sem_o):
    copies = [pltpu.make_async_copy(a, b, sem_c.at[i]) for i, (a, b) in enumerate((
        (x_hbm.at[:, SEG - PRE:, :], xq_ref),
        (prow_hbm, prow), (wr_hbm, wr_st), (wi_hbm, wi_st),
        (rowf_hbm, rowf), (mem0_hbm, mem0_ref), (x_hbm, x_ref),
        (rowg_hbm, rowg), (colf_hbm, colf), (colg_hbm, colg)))]
    first, fil, inp, tab = copies[:1], copies[1:4], copies[4:7], copies[7:]

    def pair_copies(p):
        res = [pltpu.make_async_copy(w.bitcast(U32).at[:, p, :], stage.at[j, p], sem_w.at[j, p])
               for j, w in enumerate((wq_hbm, wk_hbm, wv_hbm))]
        return res + [pltpu.make_async_copy(wo_hbm.at[p], wo_st.at[p], sem_w.at[3, p])]

    for c in first + pair_copies(0) + pair_copies(1):
        c.start()
    first[0].wait()
    xq = xq_ref[...].astype(F32).reshape(NSEG * PRE, D)
    hq[...] = pltpu.bitcast(_layernorm(xq).astype(BF16), U32)

    def weight_pair(p, _):
        for c in pair_copies(p):
            c.wait()

        @pl.when(p + 2 < NP)
        def _():
            for c in pair_copies(p + 2):
                c.start()

        @pl.when(p + 2 == NP)
        def _():
            for c in fil:
                c.start()

        for j in range(3):
            a = stage[j, p, pl.ds(0, D // 2, stride=2), :]
            b = stage[j, p, pl.ds(1, D // 2, stride=2), :]
            w = jnp.concatenate([(a & 0xFFFF) | (b << 16),
                                 (a >> 16) | (b & np.uint32(0xFFFF0000))], axis=1)
            wqkv[p, :, 256 * j:256 * (j + 1)] = w
            if j < 2:
                qk_pre[p, :, 256 * j:256 * (j + 1)] = _dot(_bf(hq[...]), _bf(w))
        wo[p] = pltpu.bitcast(wo_st[p], U32)
    with jax.named_scope("wts"):
        jax.lax.fori_loop(0, NP, weight_pair, None)

    for c in fil:
        c.wait()
    for c in inp:
        c.start()

    def filter_block(j, _):
        low = jax.lax.broadcasted_iota(jnp.int32, (128, 384), 0) % 8 < 4
        dst = pl.ds(pl.multiple_of(j * 8, 8), 8)
        for part, st in enumerate((wr_st, wi_st)):
            t = []
            for e in range(2):
                buf = wf.at[2 * part + e]
                buf[...] = st[:, pl.ds(pl.multiple_of(256 * j + 128 * e, 128), 128)].astype(F32)
                cls = [buf[pl.ds(0, 65, stride=5), :], jnp.zeros((63, 128), F32)]
                cls += [buf[pl.ds(r, 64, stride=5), :] for r in (1, 4, 2, 3)]
                w = jnp.concatenate(cls, axis=0).astype(BF16)
                t.append(_dot(_bf(prow[e]), w, _NT) * (1.0 / (S * D)))
            for e in range(2):
                w = jnp.where(low, t[e], t[1 - e])
                for c in range(3):
                    lo = 256 * c + 128 * part
                    wp[e, :, dst, lo:lo + 128] = w[:, 128 * c:128 * (c + 1)].reshape(R // 2, 8, 128)
    with jax.named_scope("filt"):
        jax.lax.fori_loop(0, S // 256, filter_block, None)

    for c in inp:
        c.wait()
    for c in tab:
        c.start()

    def quarter_rows(s):
        return pl.ds(pl.multiple_of((s % 16) * SEG, SEG), SEG)

    def spread(s, z):
        rows = quarter_rows(s)
        for q in range(4):
            t = ((s // 2) * q) % R
            zq = z if q == 0 else _rotate(z, tw[t], -tw[R + t])
            cf[q, rows, :] = zq + jnp.where(s < 16, 0.0, cf[q, rows, :])

    def after_b(s):
        rows = quarter_rows(s)
        z = ef[0, rows, :]
        for q in range(1, 4):
            t = ((s // 2) * q) % R
            z = z + _rotate(ef[q, rows, :], tw[t], tw[R + t])
        return xa[s // 16, rows, :] + _row_inv(z, rowg)

    def a_block(load, use_pre):
        x0 = load(0)

        def step(s, carry):
            mem, xs, hs, xprev = carry
            nxt = []

            def prev_fwd():
                spread(jnp.maximum(s - 1, 0), _row_fwd(xprev, rowf))

            def next_in():
                nxt.append(load(jnp.minimum(s + 1, NSEG - 1)))

            def pre(g):
                return qk_pre[g, pl.ds(pl.multiple_of(s * PRE, PRE), PRE), :]

            o = _attention_step(jnp.concatenate([mem, hs], axis=0), wqkv, wo,
                                pre if use_pre else None, (prev_fwd, next_in))
            xo = xs + o[M:]
            xa[s // 16, quarter_rows(s), :] = xo
            return o[:M], nxt[0], _layernorm(nxt[0]), xo

        init = (mem0_ref[...].astype(F32), x0, _layernorm(x0), x0)
        last = jax.lax.fori_loop(0, NSEG, step, init, unroll=UN)[3]
        spread(NSEG - 1, _row_fwd(last, rowf))

    def b_block():
        def unit(n):
            u, i = divmod(n, 8)
            q, c = divmod(u, 3)
            return u, i, q, slice(256 * c, 256 * c + 128), slice(256 * c + 128, 256 * c + 256)

        spec = {}
        for n in range(96 + 16 + BLAG):
            if n < 96:
                u, i, q, re, im = unit(n)
                rows = [slice(64 * j + 8 * i, 64 * j + 8 * i + 8) for j in range(8)]
                for m, y in enumerate(_dft8([(cf[q, r, re], cf[q, r, im]) for r in rows])):
                    yp[u, m, 8 * i:8 * i + 8, :] = _pack(*y)
            if 0 <= n - 8 < 96:
                u, m, q, re, im = unit(n - 8)
                spec[n - 8] = _dot(_bf(colf[q + 4 * m]), _bf(yp[u, m]))
            if 0 <= n - 8 - BLAG < 96:
                u, m, q, re, im = unit(n - 8 - BLAG)
                k1 = q + 4 * m
                x = spec.pop(n - 8 - BLAG)
                xr, xi = x[:64], x[64:]
                wr, wi = wp[k1 % 2, k1 // 2, :, re], wp[k1 % 2, k1 // 2, :, im]
                v = _dot(_bf(colg[k1]), _bf(_pack(xr * wr - xi * wi, xr * wi + xi * wr)))
                ef[q, 64 * m:64 * m + 64, re] = v[:64]
                ef[q, 64 * m:64 * m + 64, im] = v[64:]
            if 0 <= n - 16 - BLAG < 96:
                u, i, q, re, im = unit(n - 16 - BLAG)
                rows = [slice(64 * j + 8 * i, 64 * j + 8 * i + 8) for j in range(8)]
                y = _dft8([(ef[q, r, im], ef[q, r, re]) for r in rows])
                for r, (yi, yr) in zip(rows, y):
                    ef[q, r, re] = yr
                    ef[q, r, im] = yi

    with jax.named_scope("A1"):
        a_block(lambda s: x_ref[s].astype(F32), True)
    for c in tab:
        c.wait()
    with jax.named_scope("B1"):
        b_block()
    with jax.named_scope("A2"):
        a_block(after_b, False)
    with jax.named_scope("B2"):
        b_block()

    def out_copy(j):
        rows = pl.ds(pl.multiple_of(j * 64, 64), 64)
        return pltpu.make_async_copy(obuf.at[:, rows, :], out_hbm.at[:, rows, :], sem_o.at[j])

    def finish(j, _):
        rows = pl.ds(pl.multiple_of(j * 64, 64), 64)
        e = [ef[0, rows, :]] + [_rotate(ef[q, rows, :], tw[j * q], tw[R + j * q]) for q in range(1, 4)]
        z = [[] for _ in range(4)]
        for t in range(3):
            y = _dft4(*[(v[:, 256 * t + 128:256 * t + 256], v[:, 256 * t:256 * t + 128]) for v in e])
            for a in range(4):
                z[a] += [y[a][1], y[a][0]]
        y = _row_inv(jnp.concatenate([jnp.concatenate(za, axis=1) for za in z], axis=0), rowg)
        for a in range(4):
            obuf[a, rows, :] = (xa[a, rows, :] + y[64 * a:64 * a + 64]).astype(obuf.dtype)
        out_copy(j).start()
    with jax.named_scope("fin"):
        jax.lax.fori_loop(0, 8, finish, None)
    for j in range(8):
        out_copy(j).wait()


@functools.partial(jax.jit, static_argnames=("A_seg_len",))
def pallas_interleave_layers__memory_aug_recurrent_mem_tr__spectral_gfnet__prompt_kernel(
    A_x: jax.Array,
    A_mem0: jax.Array,
    A_Wq: jax.Array,
    A_Wk: jax.Array,
    A_Wv: jax.Array,
    A_Wo: jax.Array,
    A_seg_len: int,
    B_x: jax.Array,
    B_w_r: jax.Array,
    B_w_i: jax.Array,
):
    assert A_seg_len == SEG and A_x.shape == (1, S, D) and A_mem0.shape == (1, M, D)
    assert A_Wq.shape == (D, H, DH) and B_w_r.shape == (S, DF)
    rowf, rowg, colf, colg, prow, tw = _tables()
    hbm = pl.BlockSpec(memory_space=pltpu.HBM)
    out = pl.pallas_call(
        _kernel,
        out_shape=jax.ShapeDtypeStruct((4, S // 4, D), A_x.dtype),
        in_specs=[pl.BlockSpec(memory_space=pltpu.SMEM)] + [hbm] * 13,
        out_specs=hbm,
        scratch_shapes=[
            pltpu.VMEM((NSEG, SEG, D), BF16),
            pltpu.VMEM((NSEG, PRE, D), BF16),
            pltpu.VMEM((M, D), BF16),
            pltpu.VMEM(rowf.shape, U32),
            pltpu.VMEM(rowg.shape, U32),
            pltpu.VMEM(prow.shape, U32),
            pltpu.VMEM(colf.shape, U32),
            pltpu.VMEM(colg.shape, U32),
            pltpu.VMEM((NP, D // 2, 6 * DH), U32),
            pltpu.VMEM((NP, DH, D), U32),
            pltpu.VMEM((3, NP, D, DH), U32),
            pltpu.VMEM((NP, 2 * DH, D), BF16),
            pltpu.VMEM((DF, S), BF16),
            pltpu.VMEM((DF, S), BF16),
            pltpu.VMEM((4, DF, 128), F32),
            pltpu.VMEM((NSEG * PRE // 2, D), U32),
            pltpu.VMEM((NP, NSEG * PRE, 4 * DH), F32),
            pltpu.VMEM((4, S // 4, D), F32),
            pltpu.VMEM((4, S // 4, 768), F32),
            pltpu.VMEM((4, S // 4, 768), F32),
            pltpu.VMEM((12, 8, 64, 128), U32),
            pltpu.VMEM((2, R // 2, 64, 768), F32),
            pltpu.VMEM((4, S // 4, D), A_x.dtype),
            pltpu.SemaphoreType.DMA((4, NP)),
            pltpu.SemaphoreType.DMA((10,)),
            pltpu.SemaphoreType.DMA((8,)),
        ],
        compiler_params=pltpu.CompilerParams(vmem_limit_bytes=110 * 2 ** 20),
    )(tw, A_x.reshape(NSEG, SEG, D), A_mem0.reshape(M, D), rowf, rowg, prow, colf, colg,
      A_Wq, A_Wk, A_Wv, A_Wo.reshape(NP, 2 * DH, D), B_w_r.T, B_w_i.T)
    return out.reshape(A_x.shape)
```

```python
import functools

import numpy as np
import jax
import jax.numpy as jnp
import jax.experimental.pallas as pl
import jax.experimental.pallas.tpu as pltpu

F32 = jnp.float32
BF16 = jnp.bfloat16
U32 = jnp.uint32

S, D, DF = 2048, 640, 321
H, DH = 32, 128
M, SEG = 8, 32
L = M + SEG
NSEG = S // SEG
NP = H // 2
PRE = 8
R = 32
EPS = 1e-5

_NN = (((1,), (0,)), ((), ()))
_NT = (((1,), (1,)), ((), ()))


def _freq_classes():
    k0 = np.arange(0, DF, 5)
    k14 = np.concatenate([np.arange(1, DF, 5), np.arange(4, DF, 5)])
    k23 = np.concatenate([np.arange(2, DF, 5), np.arange(3, DF, 5)])
    return k0, k14, k23


def _tables():
    k0, k14, k23 = _freq_classes()
    b = np.arange(128)

    def ang(k):
        return 2.0 * np.pi * ((b[:, None] * k[None, :]) % D) / D

    f0 = np.zeros((128, 256))
    f0[:, :65] = np.cos(ang(k0))
    f0[:, 128:128 + 65] = -np.sin(ang(k0))
    g0 = np.zeros((256, 128))
    c0 = np.where((k0 == 0) | (k0 == D // 2), 1.0, 2.0)
    g0[:65] = (np.cos(ang(k0)) * c0).T
    g0[128:128 + 65] = (-np.sin(ang(k0)) * c0).T
    sgn = np.concatenate([np.ones(64), -np.ones(64)])[None, :]
    fs, gs = [], []
    for k in (k14, k23):
        c, s = np.cos(ang(k)), np.sin(ang(k))
        f = np.block([[c, -s], [s * sgn, c * sgn]])
        fs.append(f)
        gs.append(2.0 * f.T)
    rowf = np.concatenate([f0, fs[0], fs[1]], axis=0)
    rowg = np.concatenate([np.concatenate([g0, np.zeros((256, 128))], 1),
                           gs[0], gs[1]], axis=0)

    n2 = np.arange(64)
    colf = np.zeros((R, 128, 128))
    colg = np.zeros((R, 128, 128))
    for k1 in range(R):
        k2 = n2 ^ (4 * (k1 % 2))
        a = 2.0 * np.pi * (((k1 + R * k2)[:, None] * n2[None, :]) % S) / S
        c, s = np.cos(a), np.sin(a)
        colf[k1, :64, 0::2], colf[k1, :64, 1::2] = c, s
        colf[k1, 64:, 0::2], colf[k1, 64:, 1::2] = -s, c
        colg[k1, :64, 0::2], colg[k1, :64, 1::2] = c.T, -s.T
        colg[k1, 64:, 0::2], colg[k1, 64:, 1::2] = s.T, c.T

    prow = np.zeros((2, 128, 128))
    k1, i = b % R, b // R
    for e in range(2):
        prow[e, 8 * (k1 // 2) + 4 * ((k1 + e) % 2) + i, b] = 1.0
    tw = np.concatenate([np.cos(2 * np.pi * np.arange(R) / R), np.sin(2 * np.pi * np.arange(R) / R)])

    def words(t):
        u = np.asarray(t, np.float32).astype(BF16).view(np.uint16).astype(np.uint32)
        return u[..., 0::2, :] | (u[..., 1::2, :] << np.uint32(16))

    return words(rowf), words(rowg), words(colf), words(colg), words(prow), tw.astype(np.float32)


_C1, _C2 = float(np.cos(2 * np.pi / 5)), float(np.cos(4 * np.pi / 5))
_S1, _S2 = float(np.sin(2 * np.pi / 5)), float(np.sin(4 * np.pi / 5))
_C8 = float(np.sqrt(0.5))


def _dot(a, b, dn=_NN):
    return jax.lax.dot_general(a, b, dn, preferred_element_type=F32)


def _bf(u):
    return pltpu.bitcast(u, BF16)


def _pack(re, im):
    return pltpu.bitcast(pltpu.pack_elementwise([re, im], packed_dtype=BF16), U32)


def _layernorm(x):
    m = jnp.mean(x, axis=-1, keepdims=True)
    xc = x - m
    v = jnp.mean(xc * xc, axis=-1, keepdims=True)
    return xc * jax.lax.rsqrt(v + EPS)


def _dft4(x0, x1, x2, x3):
    ar, ai = x0[0] + x2[0], x0[1] + x2[1]
    br, bi = x0[0] - x2[0], x0[1] - x2[1]
    cr, ci = x1[0] + x3[0], x1[1] + x3[1]
    dr, di = x1[0] - x3[0], x1[1] - x3[1]
    return ((ar + cr, ai + ci), (br + di, bi - dr), (ar - cr, ai - ci), (br - di, bi + dr))


def _dft8(x):
    e = _dft4(*x[0::2])
    o = _dft4(*x[1::2])
    o1 = ((o[1][0] + o[1][1]) * _C8, (o[1][1] - o[1][0]) * _C8)
    o3 = ((o[3][1] - o[3][0]) * _C8, (o[3][0] + o[3][1]) * _C8)
    return [(e[0][0] + o[0][0], e[0][1] + o[0][1]), (e[1][0] + o1[0], e[1][1] + o1[1]),
            (e[2][0] + o[2][1], e[2][1] - o[2][0]), (e[3][0] + o3[0], e[3][1] - o3[1]),
            (e[0][0] - o[0][0], e[0][1] - o[0][1]), (e[1][0] - o1[0], e[1][1] - o1[1]),
            (e[2][0] - o[2][1], e[2][1] + o[2][0]), (e[3][0] - o3[0], e[3][1] + o3[1])]


def _rotate(z, c, s):
    res = []
    for t in range(3):
        re, im = z[:, 256 * t:256 * t + 128], z[:, 256 * t + 128:256 * t + 256]
        res += [re * c - im * s, im * c + re * s]
    return jnp.concatenate(res, axis=1)


def _row_fwd(x, rowf):
    h = _layernorm(x)
    a = [h[:, 128 * i:128 * (i + 1)] for i in range(5)]
    p1, m1, p2, m2 = a[1] + a[4], a[4] - a[1], a[2] + a[3], a[3] - a[2]
    u0 = a[0] + p1 + p2
    u1 = jnp.concatenate([a[0] + _C1 * p1 + _C2 * p2, _S1 * m1 + _S2 * m2], axis=1)
    u2 = jnp.concatenate([a[0] + _C2 * p1 + _C1 * p2, _S2 * m1 - _S1 * m2], axis=1)
    return jnp.concatenate([_dot(u0, _bf(rowf[0:64])),
                            _dot(u1, _bf(rowf[64:192])),
                            _dot(u2, _bf(rowf[192:320]))], axis=1)


def _row_inv(z, rowg):
    t0 = _dot(z[:, 0:256], _bf(rowg[0:128, 0:128]))
    t1 = _dot(z[:, 256:512], _bf(rowg[128:256]))
    t2 = _dot(z[:, 512:768], _bf(rowg[256:384]))
    t1r, t1i, t2r, t2i = t1[:, :128], t1[:, 128:], t2[:, :128], t2[:, 128:]
    a1, b1 = t0 + _C1 * t1r + _C2 * t2r, _S1 * t1i + _S2 * t2i
    a2, b2 = t0 + _C2 * t1r + _C1 * t2r, _S2 * t1i - _S1 * t2i
    return jnp.concatenate([t0 + t1r + t2r, a1 - b1, a2 - b2, a2 + b2, a1 + b1], axis=1)


def _schedule():
    order = []
    for g in range(NP):
        order += [("qkv", g), ("qk", g - 1), ("pv", g - 2)]
        if g == 6:
            order.append(("next", 0))
    order += [("wo", g) for g in range(0, 6)] + [("qk", NP - 1), ("pv", NP - 2)]
    order += [("wo", g) for g in range(6, 12)] + [("pv", NP - 1)]
    order += [("wo", g) for g in range(12, NP)] + [("prev", 0)]
    return [(op, g) for op, g in order if g >= 0]


def _attention_step(h, wqkv, wo, pre, side):
    row = jax.lax.broadcasted_iota(jnp.int32, (L, L), 0)
    col = jax.lax.broadcasted_iota(jnp.int32, (L, L), 1)
    mask = (row < M) | (row >= col)

    def project(g):
        if pre is None:
            return _dot(h, _bf(wqkv[g]))
        qk = jnp.concatenate([_dot(h[:L - PRE], _bf(wqkv[g, :, :512])), pre(g)], axis=0)
        return jnp.concatenate([qk, _dot(h, _bf(wqkv[g, :, 512:]))], axis=1)

    def scores(t):
        res = []
        for i in range(2):
            q = t[:, 128 * i:128 * i + 128]
            k = t[:, 128 * i + 256:128 * i + 384].astype(BF16)
            v = t[:, 128 * i + 512:128 * i + 640].astype(BF16)
            sc = jnp.where(mask, _dot(q, k, _NT) * (DH ** -0.5), -1e9)
            p = jnp.exp(sc - jnp.max(sc, axis=-1, keepdims=True))
            l = jnp.sum(p, axis=-1, keepdims=True)
            res.append((p, pltpu.reciprocal(l, full_range=False), v))
        return res

    qkv, prob, out, acc = {}, {}, {}, None
    for op, g in _schedule():
        if op == "qkv":
            qkv[g] = project(g)
        elif op == "qk":
            prob[g] = scores(qkv.pop(g))
        elif op == "pv":
            out[g] = jnp.concatenate([_dot(p, v) * r for p, r, v in prob.pop(g)], axis=1)
        elif op == "wo":
            d = _dot(out.pop(g), _bf(wo[g]))
            acc = d if acc is None else acc + d
        else:
            side[op]()
    return acc


def _kernel(tw, x_hbm, mem0_hbm, rowf_hbm, rowg_hbm, prow_hbm, colf_hbm, colg_hbm,
            wq_hbm, wk_hbm, wv_hbm, wo_hbm, wr_hbm, wi_hbm,
            out_hbm,
            x_ref, xq_ref, mem0_ref, rowf, rowg, prow, colf, colg,
            wqkv, wo, stage, wo_st, wr_st, wi_st, wf, hq, qk_pre,
            xa, xin, hin, cf, ef, yp, wp, obuf, sem_w, sem_f, sem_c, sem_o):
    copies = [pltpu.make_async_copy(a, b, sem_c.at[i]) for i, (a, b) in enumerate((
        (x_hbm.at[:, SEG - PRE:, :], xq_ref),
        (prow_hbm, prow),
        (rowf_hbm, rowf), (mem0_hbm, mem0_ref), (x_hbm.at[:4], x_ref.at[:4]),
        (x_hbm.at[4:], x_ref.at[4:]),
        (rowg_hbm, rowg), (colf_hbm, colf), (colg_hbm, colg)))]
    first, inp, rest, tab = copies[:2], copies[2:5], copies[5], copies[6:]

    def filter_copies(j):
        cols = pl.ds(pl.multiple_of(j * 512, 512), 512)
        return [pltpu.make_async_copy(a.at[:, cols], b.at[:, cols], sem_f.at[i, j])
                for i, (a, b) in enumerate(((wr_hbm, wr_st), (wi_hbm, wi_st)))]

    def pair_copies(p):
        res = [pltpu.make_async_copy(w.bitcast(U32).at[:, p, :], stage.at[j, p, :D], sem_w.at[j, p])
               for j, w in enumerate((wq_hbm, wk_hbm, wv_hbm))]
        return res + [pltpu.make_async_copy(wo_hbm.at[p], wo_st.at[p], sem_w.at[3, p])]

    for c in first:
        c.start()
    for c in filter_copies(0):
        c.start()
    with jax.named_scope("w_xq"):
      for c in first:
        c.wait()
    for c in filter_copies(1):
        c.start()
    with jax.named_scope("ln_xq"):
        xq = xq_ref[...].astype(F32).reshape(NSEG * PRE, D)
        hq[...] = pltpu.bitcast(_layernorm(xq).astype(BF16), U32)

    def filter_block(j):
        low = jax.lax.broadcasted_iota(jnp.int32, (128, 384), 0) % 8 < 4
        dst = pl.ds(pl.multiple_of(j * 8, 8), 8)
        for part, st in enumerate((wr_st, wi_st)):
            t = []
            for e in range(2):
                buf = wf.at[2 * part + e]
                buf[:DF] = st[:, pl.ds(pl.multiple_of(256 * j + 128 * e, 128), 128)].astype(F32)
                cls = [buf[pl.ds(0, 65, stride=5), :], jnp.zeros((63, 128), F32)]
                cls += [buf[pl.ds(r, 64, stride=5), :] for r in (1, 4, 2, 3)]
                w = jnp.concatenate(cls, axis=0).astype(BF16)
                t.append(_dot(_bf(prow[e]), w, _NT) * (1.0 / (S * D)))
            for e in range(2):
                w = jnp.where(low, t[e], t[1 - e])
                for c in range(3):
                    lo = 256 * c + 128 * part
                    wp[e, :, dst, lo:lo + 128] = w[:, 128 * c:128 * (c + 1)].reshape(R // 2, 8, 128)

    def filter_chunk(j, _):
        for c in filter_copies(j):
            c.wait()

        @pl.when(j < 2)
        def _():
            for c in filter_copies(j + 2):
                c.start()

        @pl.when(j >= 2)
        def _():
            for c in pair_copies(j - 2):
                c.start()

        filter_block(2 * j)
        filter_block(2 * j + 1)
    with jax.named_scope("filt"):
        jax.lax.fori_loop(0, 4, filter_chunk, None)

    def weight_pair(p, _):
        for c in pair_copies(p):
            c.wait()

        @pl.when(p + 2 < NP)
        def _():
            for c in pair_copies(p + 2):
                c.start()

        @pl.when(p + 2 == NP)
        def _():
            for c in inp:
                c.start()

        wo[p] = pltpu.bitcast(wo_st[p], U32)
        for j in range(3):
            a = stage[j, p, pl.ds(0, D // 2, stride=2), :]
            b = stage[j, p, pl.ds(1, D // 2, stride=2), :]
            w = jnp.concatenate([(a & 0xFFFF) | (b << 16),
                                 (a >> 16) | (b & np.uint32(0xFFFF0000))], axis=1)
            wqkv[p, :, 256 * j:256 * (j + 1)] = w
            if j < 2:
                qk_pre[p, :, 256 * j:256 * (j + 1)] = _dot(_bf(hq[...]), _bf(w))
    with jax.named_scope("wts"):
        jax.lax.fori_loop(0, NP, weight_pair, None)

    with jax.named_scope("w_inp"):
      for c in inp:
        c.wait()
    for c in [rest] + tab:
        c.start()

    def quarter_rows(s):
        return pl.ds(pl.multiple_of((s % 16) * SEG, SEG), SEG)

    def spread(s, z):
        rows = quarter_rows(s)
        for q in range(4):
            t = ((s // 2) * q) % R
            zq = z if q == 0 else _rotate(z, tw[t], -tw[R + t])
            cf[q, rows, :] = zq + jnp.where(s >= 16, cf[q, rows, :], 0.0)

    def after_b(s):
        rows = quarter_rows(s)
        z = ef[0, rows, :]
        for q in range(1, 4):
            t = ((s // 2) * q) % R
            z = z + _rotate(ef[q, rows, :], tw[t], tw[R + t])
        return xa[s // 16, rows, :] + _row_inv(z, rowg)

    def a_block(load, use_pre):
        def fetch(s, slot):
            x = load(s)
            xin[slot] = x
            hin[slot] = _layernorm(x)

        def forward(s):
            spread(s, _row_fwd(xa[s // 16, quarter_rows(s), :], rowf))

        def step(s, slot, mem):
            def pre(g):
                return qk_pre[g, pl.ds(pl.multiple_of(s * PRE, PRE), PRE), :]

            side = {"prev": lambda: forward(jnp.maximum(s - 1, 0)),
                    "next": lambda: fetch(jnp.minimum(s + 1, NSEG - 1), 1 - slot)}
            o = _attention_step(jnp.concatenate([mem, hin[slot]], axis=0), wqkv, wo,
                                pre if use_pre else None, side)
            xa[s // 16, quarter_rows(s), :] = xin[slot] + o[M:]
            return o[:M]

        def steps(t, mem):
            if use_pre:
                pl.when(t == 1)(rest.wait)
            return step(2 * t + 1, 1, step(2 * t, 0, mem))

        fetch(0, 0)
        xa[0, :SEG, :] = xin[0]
        jax.lax.fori_loop(0, NSEG // 2, steps, mem0_ref[...].astype(F32))
        forward(NSEG - 1)

    def b_block():
        def unit(n):
            u, i = divmod(n, 8)
            q, c = divmod(u, 3)
            return u, i, q, slice(256 * c, 256 * c + 128), slice(256 * c + 128, 256 * c + 256)

        spec = {}
        for n in range(96 + 18):
            if n < 96:
                u, i, q, re, im = unit(n)
                rows = [slice(64 * j + 8 * i, 64 * j + 8 * i + 8) for j in range(8)]
                for m, y in enumerate(_dft8([(cf[q, r, re], cf[q, r, im]) for r in rows])):
                    yp[u, m, 8 * i:8 * i + 8, :] = _pack(*y)
            if 0 <= n - 8 < 96:
                u, m, q, re, im = unit(n - 8)
                spec[n - 8] = _dot(_bf(colf[q + 4 * m]), _bf(yp[u, m]))
            if 0 <= n - 10 < 96:
                u, m, q, re, im = unit(n - 10)
                k1 = q + 4 * m
                x = spec.pop(n - 10)
                xr, xi = x[:64], x[64:]
                wr, wi = wp[k1 % 2, k1 // 2, :, re], wp[k1 % 2, k1 // 2, :, im]
                v = _dot(_bf(colg[k1]), _bf(_pack(xr * wr - xi * wi, xr * wi + xi * wr)))
                ef[q, 64 * m:64 * m + 64, re] = v[:64]
                ef[q, 64 * m:64 * m + 64, im] = v[64:]
            if 0 <= n - 18 < 96:
                u, i, q, re, im = unit(n - 18)
                rows = [slice(64 * j + 8 * i, 64 * j + 8 * i + 8) for j in range(8)]
                y = _dft8([(ef[q, r, im], ef[q, r, re]) for r in rows])
                for r, (yi, yr) in zip(rows, y):
                    ef[q, r, re] = yr
                    ef[q, r, im] = yi

    with jax.named_scope("A1"):
        a_block(lambda s: x_ref[s].astype(F32), True)
    with jax.named_scope("w_tab"):
      for c in tab:
        c.wait()
    with jax.named_scope("B1"):
        b_block()
    with jax.named_scope("A2"):
        a_block(after_b, False)
    with jax.named_scope("B2"):
        b_block()

    def out_copy(j):
        rows = pl.ds(pl.multiple_of(j * 64, 64), 64)
        return pltpu.make_async_copy(obuf.at[:, rows, :], out_hbm.at[:, rows, :], sem_o.at[j])

    def finish(j, _):
        rows = pl.ds(pl.multiple_of(j * 64, 64), 64)
        e = [ef[0, rows, :]] + [_rotate(ef[q, rows, :], tw[j * q], tw[R + j * q]) for q in range(1, 4)]
        z = [[] for _ in range(4)]
        for t in range(3):
            y = _dft4(*[(v[:, 256 * t + 128:256 * t + 256], v[:, 256 * t:256 * t + 128]) for v in e])
            for a in range(4):
                z[a] += [y[a][1], y[a][0]]
        y = _row_inv(jnp.concatenate([jnp.concatenate(za, axis=1) for za in z], axis=0), rowg)
        for a in range(4):
            obuf[a, rows, :] = (xa[a, rows, :] + y[64 * a:64 * a + 64]).astype(obuf.dtype)
        out_copy(j).start()
    with jax.named_scope("fin"):
        jax.lax.fori_loop(0, 8, finish, None)
    with jax.named_scope("w_out"):
      for j in range(8):
        out_copy(j).wait()


@functools.partial(jax.jit, static_argnames=("A_seg_len",))
def pallas_interleave_layers__memory_aug_recurrent_mem_tr__spectral_gfnet__prompt_kernel(
    A_x: jax.Array,
    A_mem0: jax.Array,
    A_Wq: jax.Array,
    A_Wk: jax.Array,
    A_Wv: jax.Array,
    A_Wo: jax.Array,
    A_seg_len: int,
    B_x: jax.Array,
    B_w_r: jax.Array,
    B_w_i: jax.Array,
):
    assert A_seg_len == SEG and A_x.shape == (1, S, D) and A_mem0.shape == (1, M, D)
    assert A_Wq.shape == (D, H, DH) and B_w_r.shape == (S, DF)
    rowf, rowg, colf, colg, prow, tw = _tables()
    hbm = pl.BlockSpec(memory_space=pltpu.HBM)
    out = pl.pallas_call(
        _kernel,
        out_shape=jax.ShapeDtypeStruct((4, S // 4, D), A_x.dtype),
        in_specs=[pl.BlockSpec(memory_space=pltpu.SMEM)] + [hbm] * 13,
        out_specs=hbm,
        scratch_shapes=[
            pltpu.VMEM((NSEG, SEG, D), BF16),
            pltpu.VMEM((NSEG, PRE, D), BF16),
            pltpu.VMEM((M, D), BF16),
            pltpu.VMEM(rowf.shape, U32),
            pltpu.VMEM(rowg.shape, U32),
            pltpu.VMEM(prow.shape, U32),
            pltpu.VMEM(colf.shape, U32),
            pltpu.VMEM(colg.shape, U32),
            pltpu.VMEM((NP, D // 2, 6 * DH), U32),
            pltpu.VMEM((NP, DH, D), U32),
            pltpu.VMEM((3, NP, D + 8, DH), U32),
            pltpu.VMEM((NP, 2 * DH, D), BF16),
            pltpu.VMEM((DF, S), BF16),
            pltpu.VMEM((DF, S), BF16),
            pltpu.VMEM((4, DF + 7, 128), F32),
            pltpu.VMEM((NSEG * PRE // 2, D), U32),
            pltpu.VMEM((NP, NSEG * PRE, 4 * DH), F32),
            pltpu.VMEM((4, S // 4, D), F32),
            pltpu.VMEM((2, SEG, D), F32),
            pltpu.VMEM((2, SEG, D), F32),
            pltpu.VMEM((4, S // 4, 768), F32),
            pltpu.VMEM((4, S // 4, 768), F32),
            pltpu.VMEM((12, 8, 64, 128), U32),
            pltpu.VMEM((2, R // 2, 64, 768), F32),
            pltpu.VMEM((4, S // 4, D), A_x.dtype),
            pltpu.SemaphoreType.DMA((4, NP)),
            pltpu.SemaphoreType.DMA((2, 4)),
            pltpu.SemaphoreType.DMA((9,)),
            pltpu.SemaphoreType.DMA((8,)),
        ],
        compiler_params=pltpu.CompilerParams(vmem_limit_bytes=110 * 2 ** 20),
    )(tw, A_x.reshape(NSEG, SEG, D), A_mem0.reshape(M, D), rowf, rowg, prow, colf, colg,
      A_Wq, A_Wk, A_Wv, A_Wo.reshape(NP, 2 * DH, D), B_w_r.T, B_w_i.T)
    return out.reshape(A_x.shape)
```

```python
import functools

import numpy as np
import jax
import jax.numpy as jnp
import jax.experimental.pallas as pl
import jax.experimental.pallas.tpu as pltpu

F32 = jnp.float32
BF16 = jnp.bfloat16
U32 = jnp.uint32

S, D, DF = 2048, 640, 321
H, DH = 32, 128
M, SEG = 8, 32
L = M + SEG
NSEG = S // SEG
NP = H // 2
PRE = 8
R = 32
EPS = 1e-5

_NN = (((1,), (0,)), ((), ()))
_NT = (((1,), (1,)), ((), ()))


def _freq_classes():
    k0 = np.arange(0, DF, 5)
    k14 = np.concatenate([np.arange(1, DF, 5), np.arange(4, DF, 5)])
    k23 = np.concatenate([np.arange(2, DF, 5), np.arange(3, DF, 5)])
    return k0, k14, k23


def _tables():
    k0, k14, k23 = _freq_classes()
    b = np.arange(128)

    def ang(k):
        return 2.0 * np.pi * ((b[:, None] * k[None, :]) % D) / D

    f0 = np.zeros((128, 256))
    f0[:, :65] = np.cos(ang(k0))
    f0[:, 128:128 + 65] = -np.sin(ang(k0))
    g0 = np.zeros((256, 128))
    c0 = np.where((k0 == 0) | (k0 == D // 2), 1.0, 2.0)
    g0[:65] = (np.cos(ang(k0)) * c0).T
    g0[128:128 + 65] = (-np.sin(ang(k0)) * c0).T
    sgn = np.concatenate([np.ones(64), -np.ones(64)])[None, :]
    fs, gs = [], []
    for k in (k14, k23):
        c, s = np.cos(ang(k)), np.sin(ang(k))
        f = np.block([[c, -s], [s * sgn, c * sgn]])
        fs.append(f)
        gs.append(2.0 * f.T)
    rowf = np.concatenate([f0, fs[0], fs[1]], axis=0)
    rowg = np.concatenate([np.concatenate([g0, np.zeros((256, 128))], 1),
                           gs[0], gs[1]], axis=0)

    n2 = np.arange(64)
    at = 16 * (n2 // 8) + n2 % 8
    colf = np.zeros((R, 128, 128))
    colg = np.zeros((R, 128, 128))
    for k1 in range(R):
        k2 = n2 ^ (4 * (k1 % 2))
        a = 2.0 * np.pi * (((k1 + R * k2)[:, None] * n2[None, :]) % S) / S
        c, s = np.cos(a), np.sin(a)
        colf[k1][:, np.concatenate([at, at + 8])] = np.block([[c, s], [-s, c]])
        colg[k1] = np.block([[c.T, -s.T], [s.T, c.T]])

    prow = np.zeros((2, 128, 128))
    k1, i = b % R, b // R
    for e in range(2):
        prow[e, 8 * (k1 // 2) + 4 * ((k1 + e) % 2) + i, b] = 1.0
    tw = np.concatenate([np.cos(2 * np.pi * np.arange(R) / R), np.sin(2 * np.pi * np.arange(R) / R)])

    def words(t):
        u = np.asarray(t, np.float32).astype(BF16).view(np.uint16).astype(np.uint32)
        return u[..., 0::2, :] | (u[..., 1::2, :] << np.uint32(16))

    return words(rowf), words(rowg), words(colf), words(colg), words(prow), tw.astype(np.float32)


_C1, _C2 = float(np.cos(2 * np.pi / 5)), float(np.cos(4 * np.pi / 5))
_S1, _S2 = float(np.sin(2 * np.pi / 5)), float(np.sin(4 * np.pi / 5))
_C8 = float(np.sqrt(0.5))


def _dot(a, b, dn=_NN):
    return jax.lax.dot_general(a, b, dn, preferred_element_type=F32)


def _bf(u):
    return pltpu.bitcast(u, BF16)


def _pack(re, im):
    return jnp.concatenate([re, im], axis=0).astype(BF16)


def _layernorm(x):
    m = jnp.mean(x, axis=-1, keepdims=True)
    xc = x - m
    v = jnp.mean(xc * xc, axis=-1, keepdims=True)
    return xc * jax.lax.rsqrt(v + EPS)


def _dft4(x0, x1, x2, x3):
    ar, ai = x0[0] + x2[0], x0[1] + x2[1]
    br, bi = x0[0] - x2[0], x0[1] - x2[1]
    cr, ci = x1[0] + x3[0], x1[1] + x3[1]
    dr, di = x1[0] - x3[0], x1[1] - x3[1]
    return ((ar + cr, ai + ci), (br + di, bi - dr), (ar - cr, ai - ci), (br - di, bi + dr))


def _dft8(x):
    e = _dft4(*x[0::2])
    o = _dft4(*x[1::2])
    o1 = ((o[1][0] + o[1][1]) * _C8, (o[1][1] - o[1][0]) * _C8)
    o3 = ((o[3][1] - o[3][0]) * _C8, (o[3][0] + o[3][1]) * _C8)
    return [(e[0][0] + o[0][0], e[0][1] + o[0][1]), (e[1][0] + o1[0], e[1][1] + o1[1]),
            (e[2][0] + o[2][1], e[2][1] - o[2][0]), (e[3][0] + o3[0], e[3][1] - o3[1]),
            (e[0][0] - o[0][0], e[0][1] - o[0][1]), (e[1][0] - o1[0], e[1][1] - o1[1]),
            (e[2][0] - o[2][1], e[2][1] + o[2][0]), (e[3][0] - o3[0], e[3][1] + o3[1])]


def _rotate(z, c, s):
    res = []
    for t in range(3):
        re, im = z[:, 256 * t:256 * t + 128], z[:, 256 * t + 128:256 * t + 256]
        res += [re * c - im * s, im * c + re * s]
    return jnp.concatenate(res, axis=1)


def _row_fwd(x, rowf):
    h = _layernorm(x)
    a = [h[:, 128 * i:128 * (i + 1)] for i in range(5)]
    p1, m1, p2, m2 = a[1] + a[4], a[4] - a[1], a[2] + a[3], a[3] - a[2]
    u0 = a[0] + p1 + p2
    u1 = jnp.concatenate([a[0] + _C1 * p1 + _C2 * p2, _S1 * m1 + _S2 * m2], axis=1)
    u2 = jnp.concatenate([a[0] + _C2 * p1 + _C1 * p2, _S2 * m1 - _S1 * m2], axis=1)
    return jnp.concatenate([_dot(u0, _bf(rowf[0:64])),
                            _dot(u1, _bf(rowf[64:192])),
                            _dot(u2, _bf(rowf[192:320]))], axis=1)


def _row_inv(z, rowg):
    t0 = _dot(z[:, 0:256], _bf(rowg[0:128, 0:128]))
    t1 = _dot(z[:, 256:512], _bf(rowg[128:256]))
    t2 = _dot(z[:, 512:768], _bf(rowg[256:384]))
    t1r, t1i, t2r, t2i = t1[:, :128], t1[:, 128:], t2[:, :128], t2[:, 128:]
    a1, b1 = t0 + _C1 * t1r + _C2 * t2r, _S1 * t1i + _S2 * t2i
    a2, b2 = t0 + _C2 * t1r + _C1 * t2r, _S2 * t1i - _S1 * t2i
    return jnp.concatenate([t0 + t1r + t2r, a1 - b1, a2 - b2, a2 + b2, a1 + b1], axis=1)


def _schedule():
    order = []
    for g in range(NP):
        order += [("qkv", g), ("qk", g - 1), ("pv", g - 2)]
        if g == 6:
            order.append(("next", 0))
    order += [("wo", g) for g in range(0, 6)] + [("qk", NP - 1), ("pv", NP - 2)]
    order += [("wo", g) for g in range(6, 12)] + [("pv", NP - 1)]
    order += [("wo", g) for g in range(12, NP)] + [("prev", 0)]
    return [(op, g) for op, g in order if g >= 0]


def _attention_step(h, wqkv, wo, pre, side):
    row = jax.lax.broadcasted_iota(jnp.int32, (L, L), 0)
    col = jax.lax.broadcasted_iota(jnp.int32, (L, L), 1)
    mask = (row < M) | (row >= col)

    def project(g):
        if pre is None:
            return _dot(h, _bf(wqkv[g]))
        qk = jnp.concatenate([_dot(h[:L - PRE], _bf(wqkv[g, :, :512])), pre(g)], axis=0)
        return jnp.concatenate([qk, _dot(h, _bf(wqkv[g, :, 512:]))], axis=1)

    def scores(t):
        res = []
        for i in range(2):
            q = t[:, 128 * i:128 * i + 128]
            k = t[:, 128 * i + 256:128 * i + 384].astype(BF16)
            v = t[:, 128 * i + 512:128 * i + 640].astype(BF16)
            sc = jnp.where(mask, _dot(q, k, _NT) * (DH ** -0.5), -1e9)
            p = jnp.exp(sc - jnp.max(sc, axis=-1, keepdims=True))
            l = jnp.sum(p, axis=-1, keepdims=True)
            res.append((p, pltpu.reciprocal(l, full_range=False), v))
        return res

    qkv, prob, out, acc = {}, {}, {}, None
    for op, g in _schedule():
        if op == "qkv":
            qkv[g] = project(g)
        elif op == "qk":
            prob[g] = scores(qkv.pop(g))
        elif op == "pv":
            out[g] = jnp.concatenate([_dot(p, v) * r for p, r, v in prob.pop(g)], axis=1)
        elif op == "wo":
            d = _dot(out.pop(g), _bf(wo[g]))
            acc = d if acc is None else acc + d
        else:
            side[op]()
    return acc


def _kernel(tw, x_hbm, mem0_hbm, rowf_hbm, rowg_hbm, prow_hbm, colf_hbm, colg_hbm,
            wq_hbm, wk_hbm, wv_hbm, wo_hbm, wr_hbm, wi_hbm,
            out_hbm,
            x_ref, xq_ref, mem0_ref, rowf, rowg, prow, colf, colg,
            wqkv, wo, stage, wo_st, wr_st, wi_st, wf, hq, qk_pre,
            xa, xin, hin, cf, ef, yp, wp, obuf, sem_w, sem_f, sem_c, sem_o):
    copies = [pltpu.make_async_copy(a, b, sem_c.at[i]) for i, (a, b) in enumerate((
        (x_hbm.at[:, SEG - PRE:, :], xq_ref),
        (prow_hbm, prow),
        (rowf_hbm, rowf), (mem0_hbm, mem0_ref), (x_hbm.at[:4], x_ref.at[:4]),
        (x_hbm.at[4:], x_ref.at[4:]),
        (rowg_hbm, rowg), (colf_hbm, colf), (colg_hbm, colg)))]
    first, inp, rest, tab = copies[:2], copies[2:5], copies[5], copies[6:]

    def filter_copies(j):
        cols = pl.ds(pl.multiple_of(j * 512, 512), 512)
        return [pltpu.make_async_copy(a.at[:, cols], b.at[:, cols], sem_f.at[i, j])
                for i, (a, b) in enumerate(((wr_hbm, wr_st), (wi_hbm, wi_st)))]

    def pair_copies(p):
        res = [pltpu.make_async_copy(w.bitcast(U32).at[:, p, :], stage.at[j, p, :D], sem_w.at[j, p])
               for j, w in enumerate((wq_hbm, wk_hbm, wv_hbm))]
        return res + [pltpu.make_async_copy(wo_hbm.at[p], wo_st.at[p], sem_w.at[3, p])]

    for c in first:
        c.start()
    for c in filter_copies(0):
        c.start()
    for c in first:
        c.wait()
    for c in filter_copies(1):
        c.start()
    xq = xq_ref[...].astype(F32).reshape(NSEG * PRE, D)
    hq[...] = pltpu.bitcast(_layernorm(xq).astype(BF16), U32)

    def filter_block(j):
        low = jax.lax.broadcasted_iota(jnp.int32, (128, 384), 0) % 8 < 4
        dst = pl.ds(pl.multiple_of(j * 8, 8), 8)
        for part, st in enumerate((wr_st, wi_st)):
            t = []
            for e in range(2):
                buf = wf.at[2 * part + e]
                buf[:DF] = st[:, pl.ds(pl.multiple_of(256 * j + 128 * e, 128), 128)].astype(F32)
                cls = [buf[pl.ds(0, 65, stride=5), :], jnp.zeros((63, 128), F32)]
                cls += [buf[pl.ds(r, 64, stride=5), :] for r in (1, 4, 2, 3)]
                w = jnp.concatenate(cls, axis=0).astype(BF16)
                t.append(_dot(_bf(prow[e]), w, _NT) * (1.0 / (S * D)))
            for e in range(2):
                w = jnp.where(low, t[e], t[1 - e])
                for c in range(3):
                    lo = 256 * c + 128 * part
                    wp[e, :, dst, lo:lo + 128] = w[:, 128 * c:128 * (c + 1)].reshape(R // 2, 8, 128)

    def filter_chunk(j, _):
        for c in filter_copies(j):
            c.wait()

        @pl.when(j < 2)
        def _():
            for c in filter_copies(j + 2):
                c.start()

        @pl.when(j >= 2)
        def _():
            for c in pair_copies(j - 2):
                c.start()

        filter_block(2 * j)
        filter_block(2 * j + 1)
    jax.lax.fori_loop(0, 4, filter_chunk, None)

    def weight_pair(p, _):
        for c in pair_copies(p):
            c.wait()

        @pl.when(p + 2 < NP)
        def _():
            for c in pair_copies(p + 2):
                c.start()

        @pl.when(p + 2 == NP)
        def _():
            for c in inp:
                c.start()

        wo[p] = pltpu.bitcast(wo_st[p], U32)
        for j in range(3):
            a = stage[j, p, pl.ds(0, D // 2, stride=2), :]
            b = stage[j, p, pl.ds(1, D // 2, stride=2), :]
            w = jnp.concatenate([(a & 0xFFFF) | (b << 16),
                                 (a >> 16) | (b & np.uint32(0xFFFF0000))], axis=1)
            wqkv[p, :, 256 * j:256 * (j + 1)] = w
            if j < 2:
                qk_pre[p, :, 256 * j:256 * (j + 1)] = _dot(_bf(hq[...]), _bf(w))
    jax.lax.fori_loop(0, NP, weight_pair, None)

    for c in inp:
        c.wait()
    for c in [rest] + tab:
        c.start()

    def quarter_rows(s):
        return pl.ds(pl.multiple_of((s % 16) * SEG, SEG), SEG)

    def spread(s, z):
        rows = quarter_rows(s)
        for q in range(4):
            t = ((s // 2) * q) % R
            zq = z if q == 0 else _rotate(z, tw[t], -tw[R + t])
            cf[q, rows, :] = zq + jnp.where(s >= 16, cf[q, rows, :], 0.0)

    def after_b(s):
        rows = quarter_rows(s)
        z = ef[0, rows, :]
        for q in range(1, 4):
            t = ((s // 2) * q) % R
            z = z + _rotate(ef[q, rows, :], tw[t], tw[R + t])
        return xa[s // 16, rows, :] + _row_inv(z, rowg)

    def a_block(load, use_pre):
        def fetch(s, slot):
            x = load(s)
            xin[slot] = x
            hin[slot] = _layernorm(x)

        def forward(s):
            spread(s, _row_fwd(xa[s // 16, quarter_rows(s), :], rowf))

        def step(s, slot, mem):
            def pre(g):
                return qk_pre[g, pl.ds(pl.multiple_of(s * PRE, PRE), PRE), :]

            side = {"prev": lambda: forward(jnp.maximum(s - 1, 0)),
                    "next": lambda: fetch(jnp.minimum(s + 1, NSEG - 1), 1 - slot)}
            o = _attention_step(jnp.concatenate([mem, hin[slot]], axis=0), wqkv, wo,
                                pre if use_pre else None, side)
            xa[s // 16, quarter_rows(s), :] = xin[slot] + o[M:]
            return o[:M]

        def steps(t, mem):
            if use_pre:
                pl.when(t == 1)(rest.wait)
            return step(2 * t + 1, 1, step(2 * t, 0, mem))

        fetch(0, 0)
        xa[0, :SEG, :] = xin[0]
        jax.lax.fori_loop(0, NSEG // 2, steps, mem0_ref[...].astype(F32))
        forward(NSEG - 1)

    def b_block():
        def unit(n):
            u, i = divmod(n, 8)
            q, c = divmod(u, 3)
            return u, i, q, slice(256 * c, 256 * c + 128), slice(256 * c + 128, 256 * c + 256)

        spec = {}
        for n in range(96 + 18):
            if n < 96:
                u, i, q, re, im = unit(n)
                rows = [slice(64 * j + 8 * i, 64 * j + 8 * i + 8) for j in range(8)]
                for m, y in enumerate(_dft8([(cf[q, r, re], cf[q, r, im]) for r in rows])):
                    yp[u, m, 8 * i:8 * i + 8, :] = pltpu.bitcast(_pack(*y), U32)
            if 0 <= n - 8 < 96:
                u, m, q, re, im = unit(n - 8)
                spec[n - 8] = _dot(_bf(colf[q + 4 * m]), _bf(yp[u, m]))
            if 0 <= n - 10 < 96:
                u, m, q, re, im = unit(n - 10)
                k1 = q + 4 * m
                x = spec.pop(n - 10)
                xr, xi = x[:64], x[64:]
                wr, wi = wp[k1 % 2, k1 // 2, :, re], wp[k1 % 2, k1 // 2, :, im]
                v = _dot(_bf(colg[k1]), _pack(xr * wr - xi * wi, xr * wi + xi * wr))
                ef[q, 64 * m:64 * m + 64, re] = v[:64]
                ef[q, 64 * m:64 * m + 64, im] = v[64:]
            if 0 <= n - 18 < 96:
                u, i, q, re, im = unit(n - 18)
                rows = [slice(64 * j + 8 * i, 64 * j + 8 * i + 8) for j in range(8)]
                y = _dft8([(ef[q, r, im], ef[q, r, re]) for r in rows])
                for r, (yi, yr) in zip(rows, y):
                    ef[q, r, re] = yr
                    ef[q, r, im] = yi

    a_block(lambda s: x_ref[s].astype(F32), True)
    for c in tab:
        c.wait()
    b_block()
    a_block(after_b, False)
    b_block()

    def out_copy(j):
        rows = pl.ds(pl.multiple_of(j * 64, 64), 64)
        return pltpu.make_async_copy(obuf.at[:, rows, :], out_hbm.at[:, rows, :], sem_o.at[j])

    def finish(j, _):
        rows = pl.ds(pl.multiple_of(j * 64, 64), 64)
        e = [ef[0, rows, :]] + [_rotate(ef[q, rows, :], tw[j * q], tw[R + j * q]) for q in range(1, 4)]
        z = [[] for _ in range(4)]
        for t in range(3):
            y = _dft4(*[(v[:, 256 * t + 128:256 * t + 256], v[:, 256 * t:256 * t + 128]) for v in e])
            for a in range(4):
                z[a] += [y[a][1], y[a][0]]
        y = _row_inv(jnp.concatenate([jnp.concatenate(za, axis=1) for za in z], axis=0), rowg)
        for a in range(4):
            obuf[a, rows, :] = (xa[a, rows, :] + y[64 * a:64 * a + 64]).astype(obuf.dtype)
        out_copy(j).start()
    jax.lax.fori_loop(0, 8, finish, None)
    for j in range(8):
        out_copy(j).wait()


@functools.partial(jax.jit, static_argnames=("A_seg_len",))
def pallas_interleave_layers__memory_aug_recurrent_mem_tr__spectral_gfnet__prompt_kernel(
    A_x: jax.Array,
    A_mem0: jax.Array,
    A_Wq: jax.Array,
    A_Wk: jax.Array,
    A_Wv: jax.Array,
    A_Wo: jax.Array,
    A_seg_len: int,
    B_x: jax.Array,
    B_w_r: jax.Array,
    B_w_i: jax.Array,
):
    assert A_seg_len == SEG and A_x.shape == (1, S, D) and A_mem0.shape == (1, M, D)
    assert A_Wq.shape == (D, H, DH) and B_w_r.shape == (S, DF)
    rowf, rowg, colf, colg, prow, tw = _tables()
    hbm = pl.BlockSpec(memory_space=pltpu.HBM)
    out = pl.pallas_call(
        _kernel,
        out_shape=jax.ShapeDtypeStruct((4, S // 4, D), A_x.dtype),
        in_specs=[pl.BlockSpec(memory_space=pltpu.SMEM)] + [hbm] * 13,
        out_specs=hbm,
        scratch_shapes=[
            pltpu.VMEM((NSEG, SEG, D), BF16),
            pltpu.VMEM((NSEG, PRE, D), BF16),
            pltpu.VMEM((M, D), BF16),
            pltpu.VMEM(rowf.shape, U32),
            pltpu.VMEM(rowg.shape, U32),
            pltpu.VMEM(prow.shape, U32),
            pltpu.VMEM(colf.shape, U32),
            pltpu.VMEM(colg.shape, U32),
            pltpu.VMEM((NP, D // 2, 6 * DH), U32),
            pltpu.VMEM((NP, DH, D), U32),
            pltpu.VMEM((3, NP, D + 8, DH), U32),
            pltpu.VMEM((NP, 2 * DH, D), BF16),
            pltpu.VMEM((DF, S), BF16),
            pltpu.VMEM((DF, S), BF16),
            pltpu.VMEM((4, DF + 7, 128), F32),
            pltpu.VMEM((NSEG * PRE // 2, D), U32),
            pltpu.VMEM((NP, NSEG * PRE, 4 * DH), F32),
            pltpu.VMEM((4, S // 4, D), F32),
            pltpu.VMEM((2, SEG, D), F32),
            pltpu.VMEM((2, SEG, D), F32),
            pltpu.VMEM((4, S // 4, 768), F32),
            pltpu.VMEM((4, S // 4, 768), F32),
            pltpu.VMEM((12, 8, 64, 128), U32),
            pltpu.VMEM((2, R // 2, 64, 768), F32),
            pltpu.VMEM((4, S // 4, D), A_x.dtype),
            pltpu.SemaphoreType.DMA((4, NP)),
            pltpu.SemaphoreType.DMA((2, 4)),
            pltpu.SemaphoreType.DMA((9,)),
            pltpu.SemaphoreType.DMA((8,)),
        ],
        compiler_params=pltpu.CompilerParams(vmem_limit_bytes=110 * 2 ** 20),
    )(tw, A_x.reshape(NSEG, SEG, D), A_mem0.reshape(M, D), rowf, rowg, prow, colf, colg,
      A_Wq, A_Wk, A_Wv, A_Wo.reshape(NP, 2 * DH, D), B_w_r.T, B_w_i.T)
    return out.reshape(A_x.shape)
```
